```python
import os as _os
_os.environ.setdefault("JAX_PLATFORMS", "cpu")
import jax
import jax.numpy as jnp

def _softmax(x, axis=-1):
    return jax.nn.softmax(x, axis=axis)
def _gelu(x):
    return jax.nn.gelu(x, approximate=True)
def _silu(x):
    return jax.nn.silu(x)
def _sigmoid(x):
    return jax.nn.sigmoid(x)
def _layernorm(x, axis=-1, eps=1e-5):
    m = jnp.mean(x, axis=axis, keepdims=True)
    v = jnp.var(x, axis=axis, keepdims=True)
    return (x - m) / jnp.sqrt(v + eps)
def _scatter_add(tgt, idx, src, axis=0):
    return tgt.at[idx].add(src)
def _segment_sum(src, seg, n):
    return jax.ops.segment_sum(src, seg, n)
class _Rng:
    def __init__(self, key):
        self._k = key
    def _next(self):
        self._k, sub = jax.random.split(self._k)
        return sub
    def normal(self, shape):
        return jax.random.normal(self._next(), shape, dtype=jnp.bfloat16)
    def randint(self, lo, hi, shape):
        return jax.random.randint(self._next(), shape, lo, hi, dtype=jnp.int32)
    def uniform(self, shape, lo=0.0, hi=1.0):
        return jax.random.uniform(self._next(), shape, jnp.bfloat16, lo, hi)
    def permutation(self, n):
        return jax.random.permutation(self._next(), n)


kernel_name = 'sequential_preLN__compressed_kv_cla__dense_activation_mish__decode'

def setup_inputs():
    _rng = _Rng(jax.random.key(int.from_bytes(__import__("os").urandom(4), "little")))
    _w = (lambda a: (lambda t: t.astype(jnp.bfloat16) if jnp.issubdtype(t.dtype, jnp.floating) else t)(jnp.asarray(a)))
    def _A_setup():
        B, H, Sq, Sk, D, M = 1, 32, 1, 8192, 128, 512
        Dc = 4 * D
        return {
            "x": _w((lambda *s: _rng.normal(s) * 0.05)(B, Sq, M)),
            "c_kv": _w((lambda *s: _rng.normal(s) * 0.8)(B, Sk, Dc)),
            "w_q": _w((lambda *s: _rng.normal(s) * 0.8)(M, H, D) * (M ** -0.5)),
            "w_uk": _w((lambda *s: _rng.normal(s) * 0.8)(Dc, H, D) * (Dc ** -0.5)),
            "w_uv": _w((lambda *s: _rng.normal(s) * 0.8)(Dc, H, D) * (Dc ** -0.5)),
            "w_o": _w((lambda *s: _rng.normal(s) * 0.8)(H, D, M) * ((H * D) ** -0.5)),
        }
    _A_in = _A_setup()

    def _B_setup():
        B, S, D, F = 1, 1, 512, 1376
        return {
            "x": _w((lambda *s: _rng.normal(s) * 0.05)(B, S, D)),
            "w1": _w((lambda *s: _rng.normal(s) * 0.2)(D, F) * (D ** -0.5)),
            "b1": _w((lambda *s: _rng.normal(s) * 0.05)(F)),
            "w2": _w((lambda *s: _rng.normal(s) * 0.05)(F, D) * (F ** -0.5)),
        }
    _B_in = _B_setup()

    return {
        "A_x": _A_in["x"],
        "A_c_kv": _A_in["c_kv"],
        "A_w_q": _A_in["w_q"],
        "A_w_uk": _A_in["w_uk"],
        "A_w_uv": _A_in["w_uv"],
        "A_w_o": _A_in["w_o"],
        "B_x": _B_in["x"],
        "B_w1": _B_in["w1"],
        "B_b1": _B_in["b1"],
        "B_w2": _B_in["w2"],
    }

def reference(A_x, A_c_kv, A_w_q, A_w_uk, A_w_uv, A_w_o, B_x, B_w1, B_b1, B_w2):
    def _A_ref(x, c_kv, w_q, w_uk, w_uv, w_o):
        B, Sq, M = x.shape[0], x.shape[1], x.shape[2]
        Sk = c_kv.shape[1]
        H, D = w_q.shape[1], w_q.shape[2]
        q = jnp.einsum("bqm,mhd->bhqd", x, w_q)
        k = jnp.einsum("bkc,chd->bhkd", c_kv, w_uk)
        v = jnp.einsum("bkc,chd->bhkd", c_kv, w_uv)
        scores = jnp.einsum("bhqd,bhkd->bhqk", q, k) * (D ** -0.5)
        off = Sk - Sq
        qi = jnp.arange(Sq)[:, None]
        kj = jnp.arange(Sk)[None, :]
        cmask = kj <= (qi + off)
        scores = jnp.where(cmask[None, None], scores, -1e9)
        p = _softmax(scores, axis=-1)
        ctx = jnp.einsum("bhqk,bhkd->bhqd", p, v)
        return jnp.einsum("bhqd,hdm->bqm", ctx, w_o)

    def _B_ref(x, w1, b1, w2):
        h = jnp.einsum("bsd,df->bsf", x, w1) + b1
        sp = jnp.log1p(jnp.exp(-jnp.abs(h))) + jnp.where(h > 0, h, jnp.zeros_like(h))
        act = h * jnp.tanh(sp)
        return jnp.einsum("bsf,fd->bsd", act, w2)

    x = A_x
    h = x + _A_ref(_layernorm(x, axis=-1), A_c_kv, A_w_q, A_w_uk, A_w_uv, A_w_o)
    h2 = h + _B_ref(_layernorm(h, axis=-1), B_w1, B_b1, B_w2)
    return h2
```

```python
import jax
import jax.numpy as jnp
from jax import lax
import jax.experimental.pallas as pl
import jax.experimental.pallas.tpu as pltpu

_LANES = 128
_EPS = 1e-5


def _layernorm_f32(v):
    mu = jnp.mean(v, axis=-1, keepdims=True)
    d = v - mu
    var = jnp.mean(d * d, axis=-1, keepdims=True)
    return d / jnp.sqrt(var + _EPS)


def _chunks(total, sizes):
    out, st = [], 0
    for s in sizes:
        if st >= total:
            break
        s = min(s, total - st)
        out.append((st, s))
        st += s
    if st < total:
        out.append((st, total - st))
    return out


@jax.jit
def pallas_sequential_preLN__compressed_kv_cla__dense_activation_mish__decode_kernel(
    A_x: jax.Array,
    A_c_kv: jax.Array,
    A_w_q: jax.Array,
    A_w_uk: jax.Array,
    A_w_uv: jax.Array,
    A_w_o: jax.Array,
    B_x: jax.Array,
    B_w1: jax.Array,
    B_b1: jax.Array,
    B_w2: jax.Array,
):
    del B_x
    B, Sq, M = A_x.shape
    _, Sk, Dc = A_c_kv.shape
    _, H, D = A_w_q.shape
    F = B_w1.shape[1]
    assert B == 1 and Sq == 1 and D == _LANES and M % _LANES == 0 and Dc % _LANES == 0
    assert _LANES % H == 0 or H % _LANES == 0
    scale = float(D) ** -0.5
    bf16, f32 = jnp.bfloat16, jnp.float32

    G = _LANES * H
    TK = 1024

    ckv_chunks = _chunks(Sk, [2048] * (Sk // 2048))
    wo_chunks = _chunks(H * D, [1024] * (H * D // 1024))
    f_chunks = _chunks(F, [768])
    w2_chunks = f_chunks

    n_sems = 2 + 3 + len(ckv_chunks) + len(wo_chunks) + len(f_chunks) + len(w2_chunks)

    def kernel(x_hbm, ckv_hbm, wq_hbm, wuk_hbm, wuv_hbm, wo_hbm, w1t_hbm, b1_hbm, w2_hbm,
               o_ref,
               x_v, b1_v, wq_v, wuk_v, ckv_v, wuv_v, wo_v, w1t_v, w2_v, e_v, g_v, sems):
        sem_i = [0]

        def cp(src, dst):
            c = pltpu.make_async_copy(src, dst, sems.at[sem_i[0]])
            sem_i[0] += 1
            c.start()
            return c

        def cp_rows(src, dst, chunks):
            return [cp(src.at[pl.ds(s, n)], dst.at[pl.ds(s, n)]) for s, n in chunks]

        c_x = cp(x_hbm, x_v)
        c_wq = cp(wq_hbm, wq_v)
        c_wuk = cp(wuk_hbm, wuk_v)
        c_ckv = cp_rows(ckv_hbm, ckv_v, ckv_chunks)
        c_wuv = cp(wuv_hbm, wuv_v)
        c_wo = cp_rows(wo_hbm, wo_v, wo_chunks)
        c_b1 = cp(b1_hbm, b1_v)
        c_w1 = cp_rows(w1t_hbm, w1t_v, f_chunks)
        c_w2 = cp_rows(w2_hbm, w2_v, w2_chunks)

        e_v[...] = (lax.broadcasted_iota(jnp.int32, (_LANES, G), 1) // H
                    == lax.broadcasted_iota(jnp.int32, (_LANES, G), 0)).astype(bf16)
        g_v[...] = (lax.broadcasted_iota(jnp.int32, (G, _LANES), 0) // H
                    == lax.broadcasted_iota(jnp.int32, (G, _LANES), 1)).astype(bf16)
        head_mask = (lax.broadcasted_iota(jnp.int32, (H, G), 1) % H
                     == lax.broadcasted_iota(jnp.int32, (H, G), 0))

        def per_head_contract(y, w_ref, n_c):
            acc = jnp.zeros((H, D), f32)
            for t in range(n_c // _LANES):
                yt = y[:, t * _LANES:(t + 1) * _LANES]
                xt = jnp.dot(yt, e_v[...], preferred_element_type=f32)
                xt = jnp.where(head_mask, xt, 0.0).astype(bf16)
                acc = acc + jnp.dot(xt, w_ref[pl.ds(t * G, G), :],
                                    preferred_element_type=f32)
            return acc

        c_x.wait()
        x = x_v[...].astype(f32)
        xn = _layernorm_f32(x).astype(bf16)
        c_wq.wait()
        q = per_head_contract(jnp.broadcast_to(xn, (H, M)), wq_v, M).astype(bf16)

        c_wuk.wait()
        qa_parts = []
        for t in range(Dc // _LANES):
            a = lax.dot_general(q, wuk_v[pl.ds(t * G, G), :], (((1,), (1,)), ((), ())),
                                preferred_element_type=f32)
            a = jnp.where(head_mask, a * scale, 0.0).astype(bf16)
            qa_parts.append(jnp.dot(a, g_v[...], preferred_element_type=f32))
        qa = jnp.concatenate(qa_parts, axis=1).astype(bf16)

        m_run = jnp.full((H, 1), -jnp.inf, f32)
        l_run = jnp.zeros((H, 1), f32)
        acc = jnp.zeros((H, Dc), f32)
        for (cs, cn), c_c in zip(ckv_chunks, c_ckv):
            c_c.wait()
            for ks in range(cs, cs + cn, TK):
                kn = min(TK, cs + cn - ks)
                cblk = ckv_v[pl.ds(ks, kn), :]
                s = lax.dot_general(qa, cblk, (((1,), (1,)), ((), ())),
                                    preferred_element_type=f32)
                m_new = jnp.maximum(m_run, jnp.max(s, axis=1, keepdims=True))
                alpha = jnp.exp(m_run - m_new)
                p = jnp.exp(s - m_new)
                l_run = l_run * alpha + jnp.sum(p, axis=1, keepdims=True)
                acc = acc * alpha + jnp.dot(p.astype(bf16), cblk,
                                            preferred_element_type=f32)
                m_run = m_new
        ctx_c = (acc / l_run).astype(bf16)

        c_wuv.wait()
        ctx = per_head_contract(ctx_c, wuv_v, Dc)

        o_mask = (lax.broadcasted_iota(jnp.int32, (H, H * D), 1) // D
                  == lax.broadcasted_iota(jnp.int32, (H, H * D), 0))
        xo = jnp.where(o_mask, jnp.tile(ctx, (1, H)), 0.0).astype(bf16)
        o_acc = jnp.zeros((H, M), f32)
        for (rs, rn), c_c in zip(wo_chunks, c_wo):
            c_c.wait()
            o_acc = o_acc + jnp.dot(xo[:, rs:rs + rn], wo_v[pl.ds(rs, rn), :],
                                    preferred_element_type=f32)
        h = x + jnp.sum(o_acc, axis=0, keepdims=True)

        hn = jnp.broadcast_to(_layernorm_f32(h).astype(bf16), (8, M))
        c_b1.wait()
        b1 = b1_v[...].astype(f32).reshape(1, F)
        acts = []
        for (fs, fn), c_c in zip(f_chunks, c_w1):
            c_c.wait()
            z = lax.dot_general(hn, w1t_v[pl.ds(fs, fn), :], (((1,), (1,)), ((), ())),
                                preferred_element_type=f32) + b1[:, fs:fs + fn]
            sp = jnp.log1p(jnp.exp(-jnp.abs(z))) + jnp.maximum(z, 0.0)
            acts.append((z * jnp.tanh(sp)).astype(bf16))
        y = jnp.zeros((8, M), f32)
        for (fs, fn), c_c, act in zip(w2_chunks, c_w2, acts):
            c_c.wait()
            y = y + jnp.dot(act, w2_v[pl.ds(fs, fn), :], preferred_element_type=f32)
        o_ref[...] = (h + y[0:1, :]).astype(o_ref.dtype)

    out = pl.pallas_call(
        kernel,
        out_shape=jax.ShapeDtypeStruct((1, M), A_x.dtype),
        in_specs=[pl.BlockSpec(memory_space=pl.ANY)] * 9,
        out_specs=pl.BlockSpec(memory_space=pltpu.VMEM),
        scratch_shapes=[
            pltpu.VMEM((1, M), bf16),
            pltpu.VMEM((F,), bf16),
            pltpu.VMEM((M * H, D), bf16),
            pltpu.VMEM((Dc * H, D), bf16),
            pltpu.VMEM((Sk, Dc), bf16),
            pltpu.VMEM((Dc * H, D), bf16),
            pltpu.VMEM((H * D, M), bf16),
            pltpu.VMEM((F, M), bf16),
            pltpu.VMEM((F, M), bf16),
            pltpu.VMEM((_LANES, G), bf16),
            pltpu.VMEM((G, _LANES), bf16),
            pltpu.SemaphoreType.DMA((n_sems,)),
        ],
        compiler_params=pltpu.CompilerParams(vmem_limit_bytes=64 * 1024 * 1024),
    )(
        A_x.reshape(1, M),
        A_c_kv.reshape(Sk, Dc),
        A_w_q.reshape(M * H, D),
        A_w_uk.reshape(Dc * H, D),
        A_w_uv.reshape(Dc * H, D),
        A_w_o.reshape(H * D, M),
        B_w1.T,
        B_b1,
        B_w2,
    )
    return out.reshape(B, Sq, M)
```

```python
import jax
import jax.numpy as jnp
from jax import lax
import jax.experimental.pallas as pl
import jax.experimental.pallas.tpu as pltpu

_LANES = 128
_EPS = 1e-5


def _layernorm_f32(v):
    mu = jnp.mean(v, axis=-1, keepdims=True)
    d = v - mu
    var = jnp.mean(d * d, axis=-1, keepdims=True)
    return d / jnp.sqrt(var + _EPS)


def _chunks(total, sizes):
    out, st = [], 0
    for s in sizes:
        if st >= total:
            break
        s = min(s, total - st)
        out.append((st, s))
        st += s
    if st < total:
        out.append((st, total - st))
    return out


@jax.jit
def pallas_sequential_preLN__compressed_kv_cla__dense_activation_mish__decode_kernel(
    A_x: jax.Array,
    A_c_kv: jax.Array,
    A_w_q: jax.Array,
    A_w_uk: jax.Array,
    A_w_uv: jax.Array,
    A_w_o: jax.Array,
    B_x: jax.Array,
    B_w1: jax.Array,
    B_b1: jax.Array,
    B_w2: jax.Array,
):
    del B_x
    B, Sq, M = A_x.shape
    _, Sk, Dc = A_c_kv.shape
    _, H, D = A_w_q.shape
    F = B_w1.shape[1]
    assert B == 1 and Sq == 1 and D == _LANES and M % _LANES == 0 and Dc % _LANES == 0
    assert _LANES % H == 0 or H % _LANES == 0
    scale = float(D) ** -0.5
    bf16, f32 = jnp.bfloat16, jnp.float32

    G = _LANES * H
    TK = 1024

    ckv_chunks = _chunks(Sk, [Sk // 2])
    w2_chunks = _chunks(F, [1024])
    assert len(ckv_chunks) == 2 and len(w2_chunks) == 2
    n_sems = 3

    def kernel(x_hbm, ckv_hbm, wq_hbm, wuk_hbm, wuv_hbm, wo_hbm, w1t_hbm, b1_hbm, w2_hbm,
               o_ref,
               x_v, b1_v, wq_v, wuk_v, ckv_v, wuv_v, wo_v, w1t_v, w2_v, e_v, g_v,
               acc_v, ml_v, xo_v, h_v, hn_v, act_v, sems):
        def rows(ref, c):
            return ref.at[pl.ds(c[0], c[1])]

        group_pairs = [
            [(x_hbm, x_v), (wq_hbm, wq_v), (wuk_hbm, wuk_v)],
            [(rows(ckv_hbm, ckv_chunks[0]), rows(ckv_v, ckv_chunks[0]))],
            [(rows(ckv_hbm, ckv_chunks[1]), rows(ckv_v, ckv_chunks[1])), (wuv_hbm, wuv_v)],
            [(wo_hbm, wo_v)],
            [(b1_hbm, b1_v), (w1t_hbm, w1t_v)],
        ] + [[(rows(w2_hbm, c), rows(w2_v, c))] for c in w2_chunks]
        groups = [
            [pltpu.make_async_copy(s_, d_, sems.at[gi % n_sems]) for s_, d_ in pairs]
            for gi, pairs in enumerate(group_pairs)
        ]

        def start_group(gi):
            if gi < len(groups):
                for c in groups[gi]:
                    c.start()

        def wait_group(gi):
            for c in groups[gi]:
                c.wait()
            start_group(gi + n_sems)

        for gi in range(n_sems):
            start_group(gi)

        e_v[...] = (lax.broadcasted_iota(jnp.int32, (_LANES, G), 1) // H
                    == lax.broadcasted_iota(jnp.int32, (_LANES, G), 0)).astype(bf16)
        g_v[...] = (lax.broadcasted_iota(jnp.int32, (G, _LANES), 0) // H
                    == lax.broadcasted_iota(jnp.int32, (G, _LANES), 1)).astype(bf16)
        head_mask = (lax.broadcasted_iota(jnp.int32, (H, G), 1) % H
                     == lax.broadcasted_iota(jnp.int32, (H, G), 0))

        def per_head_contract(y, w_ref, n_c):
            acc = jnp.zeros((H, D), f32)
            for t in range(n_c // _LANES):
                yt = y[:, t * _LANES:(t + 1) * _LANES]
                xt = jnp.dot(yt, e_v[...], preferred_element_type=f32)
                xt = jnp.where(head_mask, xt, 0.0).astype(bf16)
                acc = acc + jnp.dot(xt, w_ref[pl.ds(t * G, G), :],
                                    preferred_element_type=f32)
            return acc

        wait_group(0)
        x = x_v[...].astype(f32)
        xn = _layernorm_f32(x).astype(bf16)
        q = per_head_contract(jnp.broadcast_to(xn, (H, M)), wq_v, M).astype(bf16)

        qa_parts = []
        for t in range(Dc // _LANES):
            a = lax.dot_general(q, wuk_v[pl.ds(t * G, G), :], (((1,), (1,)), ((), ())),
                                preferred_element_type=f32)
            a = jnp.where(head_mask, a * scale, 0.0).astype(bf16)
            qa_parts.append(jnp.dot(a, g_v[...], preferred_element_type=f32))
        qa = jnp.concatenate(qa_parts, axis=1).astype(bf16)

        m_run = jnp.full((H, 1), -jnp.inf, f32)
        l_run = jnp.zeros((H, 1), f32)
        acc = jnp.zeros((H, Dc), f32)
        for ci, (cs, cn) in enumerate(ckv_chunks):
            if ci > 0:
                acc_v[...] = acc
                ml_v[0] = m_run
                ml_v[1] = l_run
            wait_group(1 + ci)
            if ci > 0:
                acc, m_run, l_run = acc_v[...], ml_v[0], ml_v[1]
            for ks in range(cs, cs + cn, TK):
                kn = min(TK, cs + cn - ks)
                cblk = ckv_v[pl.ds(ks, kn), :]
                s = lax.dot_general(qa, cblk, (((1,), (1,)), ((), ())),
                                    preferred_element_type=f32)
                m_new = jnp.maximum(m_run, jnp.max(s, axis=1, keepdims=True))
                alpha = jnp.exp(m_run - m_new)
                p = jnp.exp(s - m_new)
                l_run = l_run * alpha + jnp.sum(p, axis=1, keepdims=True)
                acc = acc * alpha + jnp.dot(p.astype(bf16), cblk,
                                            preferred_element_type=f32)
                m_run = m_new
        ctx_c = (acc / l_run).astype(bf16)

        ctx = per_head_contract(ctx_c, wuv_v, Dc)

        o_mask = (lax.broadcasted_iota(jnp.int32, (H, H * D), 1) // D
                  == lax.broadcasted_iota(jnp.int32, (H, H * D), 0))
        xo_v[...] = jnp.where(o_mask, jnp.tile(ctx, (1, H)), 0.0).astype(bf16)
        wait_group(3)
        o_acc = jnp.dot(xo_v[...], wo_v[...], preferred_element_type=f32)
        h = x + jnp.sum(o_acc, axis=0, keepdims=True)

        h_v[...] = h
        hn_v[...] = jnp.broadcast_to(_layernorm_f32(h).astype(bf16), (8, M))
        wait_group(4)
        b1 = b1_v[...].astype(f32).reshape(1, F)
        z = lax.dot_general(hn_v[...], w1t_v[...], (((1,), (1,)), ((), ())),
                            preferred_element_type=f32) + b1
        sp = jnp.log1p(jnp.exp(-jnp.abs(z))) + jnp.maximum(z, 0.0)
        act_v[...] = (z * jnp.tanh(sp)).astype(bf16)
        (f0, n0), (f1, n1) = w2_chunks
        wait_group(5)
        y0 = jnp.dot(act_v[:, pl.ds(f0, n0)], w2_v[pl.ds(f0, n0), :],
                     preferred_element_type=f32)
        h_v[...] = h_v[...] + y0[0:1, :]
        wait_group(6)
        y1 = jnp.dot(act_v[:, pl.ds(f1, n1)], w2_v[pl.ds(f1, n1), :],
                     preferred_element_type=f32)
        o_ref[...] = (h_v[...] + y1[0:1, :]).astype(o_ref.dtype)

    out = pl.pallas_call(
        kernel,
        out_shape=jax.ShapeDtypeStruct((1, M), A_x.dtype),
        in_specs=[pl.BlockSpec(memory_space=pl.ANY)] * 9,
        out_specs=pl.BlockSpec(memory_space=pltpu.VMEM),
        scratch_shapes=[
            pltpu.VMEM((1, M), bf16),
            pltpu.VMEM((F,), bf16),
            pltpu.VMEM((M * H, D), bf16),
            pltpu.VMEM((Dc * H, D), bf16),
            pltpu.VMEM((Sk, Dc), bf16),
            pltpu.VMEM((Dc * H, D), bf16),
            pltpu.VMEM((H * D, M), bf16),
            pltpu.VMEM((F, M), bf16),
            pltpu.VMEM((F, M), bf16),
            pltpu.VMEM((_LANES, G), bf16),
            pltpu.VMEM((G, _LANES), bf16),
            pltpu.VMEM((H, Dc), f32),
            pltpu.VMEM((2, H, 1), f32),
            pltpu.VMEM((H, H * D), bf16),
            pltpu.VMEM((1, M), f32),
            pltpu.VMEM((8, M), bf16),
            pltpu.VMEM((8, F), bf16),
            pltpu.SemaphoreType.DMA((n_sems,)),
        ],
        compiler_params=pltpu.CompilerParams(vmem_limit_bytes=64 * 1024 * 1024),
    )(
        A_x.reshape(1, M),
        A_c_kv.reshape(Sk, Dc),
        A_w_q.reshape(M * H, D),
        A_w_uk.reshape(Dc * H, D),
        A_w_uv.reshape(Dc * H, D),
        A_w_o.reshape(H * D, M),
        B_w1.T,
        B_b1,
        B_w2,
    )
    return out.reshape(B, Sq, M)
```
